```python
import os as _os
_os.environ.setdefault("JAX_PLATFORMS", "cpu")
import jax
import jax.numpy as jnp

def _softmax(x, axis=-1):
    return jax.nn.softmax(x, axis=axis)
def _gelu(x):
    return jax.nn.gelu(x, approximate=True)
def _silu(x):
    return jax.nn.silu(x)
def _sigmoid(x):
    return jax.nn.sigmoid(x)
def _layernorm(x, axis=-1, eps=1e-5):
    m = jnp.mean(x, axis=axis, keepdims=True)
    v = jnp.var(x, axis=axis, keepdims=True)
    return (x - m) / jnp.sqrt(v + eps)
def _scatter_add(tgt, idx, src, axis=0):
    return tgt.at[idx].add(src)
def _segment_sum(src, seg, n):
    return jax.ops.segment_sum(src, seg, n)
class _Rng:
    def __init__(self, key):
        self._k = key
    def _next(self):
        self._k, sub = jax.random.split(self._k)
        return sub
    def normal(self, shape):
        return jax.random.normal(self._next(), shape, dtype=jnp.bfloat16)
    def randint(self, lo, hi, shape):
        return jax.random.randint(self._next(), shape, lo, hi, dtype=jnp.int32)
    def uniform(self, shape, lo=0.0, hi=1.0):
        return jax.random.uniform(self._next(), shape, jnp.bfloat16, lo, hi)
    def permutation(self, n):
        return jax.random.permutation(self._next(), n)


kernel_name = 'sequential_preLN__linear_attn_block__dense_activation_squared_relu__prompt'

def setup_inputs():
    _rng = _Rng(jax.random.key(int.from_bytes(__import__("os").urandom(4), "little")))
    _w = (lambda a: (lambda t: t.astype(jnp.bfloat16) if jnp.issubdtype(t.dtype, jnp.floating) else t)(jnp.asarray(a)))
    def _A_setup():
        B, S, D = 1, 2048, 576
        return {
            "x": _w((lambda *s: _rng.normal(s) * 0.05)(B, S, D)),
            "wqkv": _w((lambda *s: _rng.normal(s) * 0.1)(D, 3 * D)),
            "wo": _w((lambda *s: _rng.normal(s) * 0.05)(D, D)),
        }
    _A_in = _A_setup()

    def _B_setup():
        B, S, D, F = 1, 2048, 576, 4608
        return {
            "x": _w((lambda *s: _rng.normal(s) * 0.05)(B, S, D)),
            "w1": _w((lambda *s: _rng.normal(s) * 0.05)(D, F)),
            "b1": _w((lambda *s: _rng.normal(s) * 0.05)(F)),
            "w2": _w((lambda *s: _rng.normal(s) * 0.05)(F, D)),
            "b2": _w((lambda *s: _rng.normal(s) * 0.05)(D)),
        }
    _B_in = _B_setup()

    return {
        "A_x": _A_in["x"],
        "A_wqkv": _A_in["wqkv"],
        "A_wo": _A_in["wo"],
        "B_x": _B_in["x"],
        "B_w1": _B_in["w1"],
        "B_b1": _B_in["b1"],
        "B_w2": _B_in["w2"],
        "B_b2": _B_in["b2"],
    }

def reference(A_x, A_wqkv, A_wo, B_x, B_w1, B_b1, B_w2, B_b2):
    def _A_ref(x, wqkv, wo):
        B, S, D = x.shape
        H = 32; Dh = D // H
        qkv = (lambda x, *d: x.transpose(*d))((x @ wqkv).reshape(B, S, 3, H, Dh), 2, 0, 3, 1, 4)
        q, k, v = qkv[0], qkv[1], qkv[2]
        phi = lambda t: jnp.where(t > 0, t + 1, jnp.exp(t)) + 1e-6
        pq, pk = phi(q), phi(k)
        kv = jnp.einsum("bhsd,bhse->bhde", pk, v)
        z = jnp.einsum("bhsd->bhd", pk)
        num = jnp.einsum("bhqd,bhde->bhqe", pq, kv)
        den = jnp.einsum("bhqd,bhd->bhq", pq, z)[..., None] + 1e-6
        o = num / den
        return (lambda x, *d: x.transpose(*d))(o, 0, 2, 1, 3).reshape(B, S, D) @ wo

    def _B_ref(x, w1, b1, w2, b2):
        h = jnp.einsum("bsd,df->bsf", x, w1) + b1
        zero = jnp.zeros_like(h)
        r = jnp.where(h > zero, h, zero)
        h = r * r
        out = jnp.einsum("bsf,fd->bsd", h, w2) + b2
        return out

    x = A_x
    h = x + _A_ref(_layernorm(x, axis=-1), A_wqkv, A_wo)
    h2 = h + _B_ref(_layernorm(h, axis=-1), B_w1, B_b1, B_w2, B_b2)
    return h2
```

```python
import jax
import jax.numpy as jnp
from jax import lax
import jax.experimental.pallas as pl
import jax.experimental.pallas.tpu as pltpu

S = 2048
D = 576
F = 4608
H = 32
DH = D // H
DP = 640
LN_EPS = 1e-5
PHI_EPS = 1e-6

TS1 = 512
TSA = 512
TSF = 1024
TF = 1152

NB1 = S // TS1
NBA = S // TSA
NBF = S // TSF
NF = F // TF
ONES_ROWS = 16

_f32 = jnp.float32
_bf16 = jnp.bfloat16
_NT = (((1,), (1,)), ((), ()))


def _layernorm_t(xt):
    m = jnp.mean(xt, axis=0, keepdims=True)
    xc = xt - m
    v = jnp.mean(xc * xc, axis=0, keepdims=True)
    return xc * lax.rsqrt(v + LN_EPS)


def _head_of(idx):
    return jnp.floor((idx.astype(_f32) + 0.5) * (1.0 / DH)).astype(jnp.int32)


def _kernel(xt_hbm, wqkv_hbm, wo_hbm, w1_hbm, b1_ref, w2t_hbm, b2_ref, ot_hbm,
            xt_v, wqkv_v, wqkvt_v, wo_v, w1_v, w2t_v, pqt_v, ot_v, gt_v, mt_v, zh_v, et_v, b2c_v,
            ln2_v, acc_v,
            sem_x, sem_w, sem_o):
    def x_copy(i):
        return pltpu.make_async_copy(
            xt_hbm.at[:, pl.ds(i * TS1, TS1)], xt_v.at[:, pl.ds(i * TS1, TS1)], sem_x.at[i])

    def o_copy(i):
        return pltpu.make_async_copy(
            ot_v.at[:, pl.ds(i * TSF, TSF)], ot_hbm.at[:, pl.ds(i * TSF, TSF)], sem_o.at[i])

    wqkv_copy = pltpu.make_async_copy(wqkv_hbm, wqkv_v, sem_w.at[0])
    wo_copy = pltpu.make_async_copy(wo_hbm, wo_v, sem_w.at[1])
    w1_copy = pltpu.make_async_copy(w1_hbm, w1_v.at[pl.ds(0, D), :], sem_w.at[2])
    w2_copy = pltpu.make_async_copy(w2t_hbm, w2t_v, sem_w.at[3])

    wqkv_copy.start()
    x_copy(0).start()

    gt_v[...] = jnp.zeros(gt_v.shape, _f32)
    brow = lax.broadcasted_iota(jnp.int32, (DP - D, F), 0)
    w1_v[D:, :] = jnp.where(brow == 0, jnp.broadcast_to(b1_ref[...].astype(_f32), (DP - D, F)),
                            0.0).astype(_bf16)
    b2pad = jnp.concatenate([b2_ref[...].astype(_f32), jnp.zeros((1, DP - D), _f32)], axis=1)
    b2c_v[...] = jnp.transpose(jnp.broadcast_to(b2pad, (128, DP)))[:D, :]

    with jax.named_scope('wait_wqkv'):
        wqkv_copy.wait()
    for i in range(1, NB1):
        x_copy(i).start()
    wo_copy.start()
    w1_copy.start()
    w2_copy.start()

    with jax.named_scope('wqkv_T'):
        eye_r = lax.broadcasted_iota(jnp.int32, (128, 128), 0)
        eye_c = lax.broadcasted_iota(jnp.int32, (128, 128), 1)
        eye = jnp.where(eye_r == eye_c, 1.0, 0.0).astype(_bf16)
        for c in range(0, 3 * D, 128):
            w = min(128, 3 * D - c)
            t = lax.dot_general(eye[:w, :w], wqkv_v[:, c:c + w], _NT, preferred_element_type=_f32)
            wqkvt_v[c:c + w, :] = t.astype(_bf16)

    def phase1(i, carry):
        x_copy(i).wait()
        c0 = pl.multiple_of(i * TS1, TS1)
        xt = xt_v[:, pl.ds(c0, TS1)].astype(_f32)
        lnt = _layernorm_t(xt).astype(_bf16)
        qkvt = jnp.dot(wqkvt_v[...], lnt, preferred_element_type=_f32)
        qk = qkvt[:2 * D]
        p = (jnp.where(qk > 0, qk + 1.0, jnp.exp(qk)) + PHI_EPS).astype(_bf16)
        pqt_v[:, pl.ds(c0, TS1)] = p[:D]
        pkt = p[D:]
        vt = jnp.concatenate([qkvt[2 * D:].astype(_bf16), jnp.ones((ONES_ROWS, TS1), _bf16)], axis=0)
        gt_v[...] += lax.dot_general(vt, pkt, _NT, preferred_element_type=_f32)
        return carry

    with jax.named_scope('phase1'):
        lax.fori_loop(0, NB1, phase1, 0)

    with jax.named_scope('phase15'):
        wo_copy.wait()
        row = lax.broadcasted_iota(jnp.int32, (D, D), 0)
        col = lax.broadcasted_iota(jnp.int32, (D, D), 1)
        kvt = jnp.where(_head_of(row) == _head_of(col), gt_v[:D, :], 0.0).astype(_bf16)
        mt = lax.dot_general(wo_v[...], kvt, (((0,), (0,)), ((), ())), preferred_element_type=_f32)
        mt_v[...] = mt.astype(_bf16)

        zrow = gt_v[D:D + 1, :]
        row = lax.broadcasted_iota(jnp.int32, (H, D), 0)
        col = lax.broadcasted_iota(jnp.int32, (H, D), 1)
        zh_v[...] = jnp.where(_head_of(col) == row, jnp.broadcast_to(zrow, (H, D)), 0.0).astype(_bf16)

        row = lax.broadcasted_iota(jnp.int32, (D, 2 * H), 0)
        col = lax.broadcasted_iota(jnp.int32, (D, 2 * H), 1)
        et_v[...] = jnp.where(_head_of(row) == (col & (H - 1)), 1.0, 0.0).astype(_bf16)

    def phase2a(i, carry):
        c0 = pl.multiple_of(i * TSA, TSA)
        pqt = pqt_v[:, pl.ds(c0, TSA)]
        den = jnp.dot(zh_v[...], pqt, preferred_element_type=_f32) + PHI_EPS
        rec = 1.0 / den
        hi = rec.astype(_bf16)
        lo = (rec - hi.astype(_f32)).astype(_bf16)
        hl = jnp.concatenate([hi, lo], axis=0)
        rexp = jnp.dot(et_v[...], hl, preferred_element_type=_f32)
        at = (pqt.astype(_f32) * rexp).astype(_bf16)
        attn = jnp.dot(mt_v[...], at, preferred_element_type=_f32)
        ht = xt_v[:, pl.ds(c0, TSA)].astype(_f32) + attn
        b2c = jnp.concatenate([b2c_v[...]] * (TSA // 128), axis=1)
        acc_v[:, pl.ds(c0, TSA)] = ht + b2c
        lnt = _layernorm_t(ht)
        prow = lax.broadcasted_iota(jnp.int32, (DP - D, TSA), 0)
        lnt = jnp.concatenate([lnt, jnp.where(prow == 0, 1.0, 0.0)], axis=0)
        ln2_v[pl.ds(c0, TSA), :] = jnp.transpose(lnt).astype(_bf16)
        return carry

    with jax.named_scope('phase2a'):
        lax.fori_loop(0, NBA, phase2a, 0)

    with jax.named_scope('wait_w12'):
        w1_copy.wait()
        w2_copy.wait()

    def ffn_block(i, carry):
        r0 = pl.multiple_of(i * TSF, TSF)

        def ffn(c, carry2):
            f0 = pl.multiple_of(c * TF, TF)
            hp = jnp.dot(ln2_v[pl.ds(r0, TSF), :], w1_v[:, pl.ds(f0, TF)],
                         preferred_element_type=_f32)
            r = jnp.maximum(hp, 0.0)
            hid = (r * r).astype(_bf16)
            acc_v[:, pl.ds(r0, TSF)] += lax.dot_general(w2t_v[:, pl.ds(f0, TF)], hid, _NT,
                                                        preferred_element_type=_f32)
            return carry2

        lax.fori_loop(0, NF, ffn, 0)
        ot_v[:, pl.ds(r0, TSF)] = acc_v[:, pl.ds(r0, TSF)].astype(_bf16)
        o_copy(i).start()
        return carry

    with jax.named_scope('ffn'):
        lax.fori_loop(0, NBF, ffn_block, 0)

    with jax.named_scope('wait_out'):
        for i in range(NBF):
            o_copy(i).wait()


@jax.jit
def pallas_sequential_preLN__linear_attn_block__dense_activation_squared_relu__prompt_kernel(
    A_x, A_wqkv, A_wo, B_x, B_w1, B_b1, B_w2, B_b2):
    del B_x
    xt = jnp.transpose(A_x.reshape(S, D))
    w2t = jnp.transpose(B_w2)
    b1 = B_b1.reshape(1, F)
    b2 = B_b2.reshape(1, D)

    hbm_spec = pl.BlockSpec(memory_space=pltpu.HBM)
    vmem_spec = pl.BlockSpec(memory_space=pltpu.VMEM)

    outt = pl.pallas_call(
        _kernel,
        out_shape=jax.ShapeDtypeStruct((D, S), _bf16),
        in_specs=[hbm_spec, hbm_spec, hbm_spec, hbm_spec, vmem_spec, hbm_spec, vmem_spec],
        out_specs=hbm_spec,
        scratch_shapes=[
            pltpu.VMEM((D, S), _bf16),
            pltpu.VMEM((D, 3 * D), _bf16),
            pltpu.VMEM((3 * D, D), _bf16),
            pltpu.VMEM((D, D), _bf16),
            pltpu.VMEM((DP, F), _bf16),
            pltpu.VMEM((D, F), _bf16),
            pltpu.VMEM((D, S), _bf16),
            pltpu.VMEM((D, S), _bf16),
            pltpu.VMEM((D + ONES_ROWS, D), _f32),
            pltpu.VMEM((D, D), _bf16),
            pltpu.VMEM((H, D), _bf16),
            pltpu.VMEM((D, 2 * H), _bf16),
            pltpu.VMEM((D, 128), _f32),
            pltpu.VMEM((S, DP), _bf16),
            pltpu.VMEM((D, S), _f32),
            pltpu.SemaphoreType.DMA((NB1,)),
            pltpu.SemaphoreType.DMA((4,)),
            pltpu.SemaphoreType.DMA((NBF,)),
        ],
        compiler_params=pltpu.CompilerParams(vmem_limit_bytes=100 * 1024 * 1024),
    )(xt, A_wqkv, A_wo, B_w1, b1, w2t, b2)
    return jnp.transpose(outt).reshape(1, S, D)
```

```python
import jax
import jax.numpy as jnp
from jax import lax
import jax.experimental.pallas as pl
import jax.experimental.pallas.tpu as pltpu

S = 2048
D = 576
F = 4608
H = 32
DH = D // H
DP = 640
LN_EPS = 1e-5
PHI_EPS = 1e-6

TS1 = 512
TSA = 2048
TSF = 512

NB1 = S // TS1
NBA = S // TSA
NBF = S // TSF
ONES_ROWS = 16

_PIECES = []
for _b in range(0, D, 128):
    _w = min(128, D - _b)
    _lo = ((_b // DH) * DH) // 16 * 16
    _hi = -(-((((_b + _w - 1) // DH) + 1) * DH) // 16) * 16
    _PIECES.append((_b, _w, _lo, _hi))
_PROWS = max(hi - lo for _, _, lo, hi in _PIECES) + ONES_ROWS
_WCH = [(c, min(512, 3 * D - c)) for c in range(0, 3 * D, 512)]

_f32 = jnp.float32
_bf16 = jnp.bfloat16
_NT = (((1,), (1,)), ((), ()))
_TN = (((0,), (0,)), ((), ()))


def _layernorm_t(xt):
    m = jnp.mean(xt, axis=0, keepdims=True)
    xc = xt - m
    v = jnp.mean(xc * xc, axis=0, keepdims=True)
    return xc * lax.rsqrt(v + LN_EPS)


def _head_of(idx):
    return jnp.floor((idx.astype(_f32) + 0.5) * (1.0 / DH)).astype(jnp.int32)


def _kernel(xt_hbm, wqkv_hbm, wo_hbm, w1_hbm, b1_ref, w2t_hbm, b2_ref, ot_hbm,
            xt_v, wqkv_v, wqkvt_v, wo_v, w1_v, w2t_v, pqt_v, ot_v, gt_v, mt_v, zh_v, et_v, b2c_v,
            ln2_v, res_v,
            sem_x, sem_w, sem_o, sem_q):
    def x_copy(i):
        return pltpu.make_async_copy(
            xt_hbm.at[:, pl.ds(i * TS1, TS1)], xt_v.at[:, pl.ds(i * TS1, TS1)], sem_x.at[i])

    def o_copy(i):
        return pltpu.make_async_copy(
            ot_v.at[:, pl.ds(i * TSF, TSF)], ot_hbm.at[:, pl.ds(i * TSF, TSF)], sem_o.at[i])

    def wqkv_copy(j):
        c, w = _WCH[j]
        return pltpu.make_async_copy(
            wqkv_hbm.at[:, pl.ds(c, w)], wqkv_v.at[:, pl.ds(c, w)], sem_q.at[j])

    wo_copy = pltpu.make_async_copy(wo_hbm, wo_v, sem_w.at[0])
    w1_copy = pltpu.make_async_copy(w1_hbm, w1_v.at[pl.ds(0, D), :], sem_w.at[1])
    w2_copy = pltpu.make_async_copy(w2t_hbm, w2t_v, sem_w.at[2])

    for j in range(len(_WCH)):
        wqkv_copy(j).start()
    x_copy(0).start()

    gt_v[...] = jnp.zeros(gt_v.shape, _f32)
    brow = lax.broadcasted_iota(jnp.int32, (DP - D, F), 0)
    w1_v[D:, :] = jnp.where(
        brow == 0, jnp.broadcast_to(b1_ref[...].astype(_f32).reshape(1, F), (DP - D, F)),
        0.0).astype(_bf16)
    b2pad = jnp.concatenate(
        [b2_ref[...].astype(_f32).reshape(1, D), jnp.zeros((1, DP - D), _f32)], axis=1)
    b2c_v[...] = jnp.transpose(jnp.broadcast_to(b2pad, (128, DP)))[:D, :]

    eye_r = lax.broadcasted_iota(jnp.int32, (128, 128), 0)
    eye_c = lax.broadcasted_iota(jnp.int32, (128, 128), 1)
    eye = jnp.where(eye_r == eye_c, 1.0, 0.0).astype(_bf16)
    for j, (c0, wc) in enumerate(_WCH):
        wqkv_copy(j).wait()
        if j == len(_WCH) - 1:
            for i in range(1, NB1):
                x_copy(i).start()
            wo_copy.start()
            w1_copy.start()
            w2_copy.start()
        for c in range(c0, c0 + wc, 128):
            w = min(128, 3 * D - c)
            t = lax.dot_general(eye[:w, :w], wqkv_v[:, c:c + w], _NT, preferred_element_type=_f32)
            wqkvt_v[c:c + w, :] = t.astype(_bf16)

    def phase1(i, carry):
        x_copy(i).wait()
        c0 = pl.multiple_of(i * TS1, TS1)
        xt = xt_v[:, pl.ds(c0, TS1)].astype(_f32)
        lnt = _layernorm_t(xt).astype(_bf16)
        qkvt = jnp.dot(wqkvt_v[...], lnt, preferred_element_type=_f32)
        qk = qkvt[:2 * D]
        p = (jnp.where(qk > 0, qk + 1.0, jnp.exp(qk)) + PHI_EPS).astype(_bf16)
        pqt_v[:, pl.ds(c0, TS1)] = p[:D]
        pkt = p[D:]
        vt = qkvt[2 * D:].astype(_bf16)
        ones = jnp.ones((ONES_ROWS, TS1), _bf16)
        for b, (d0, w, lo, hi) in enumerate(_PIECES):
            lhs = jnp.concatenate([vt[lo:hi], ones], axis=0)
            gt_v[b, :hi - lo + ONES_ROWS, :w] += lax.dot_general(
                lhs, pkt[d0:d0 + w], _NT, preferred_element_type=_f32)
        return carry

    lax.fori_loop(0, NB1, phase1, 0)

    wo_copy.wait()
    for b, (d0, w, lo, hi) in enumerate(_PIECES):
        n = hi - lo
        row = lax.broadcasted_iota(jnp.int32, (n, w), 0) + lo
        col = lax.broadcasted_iota(jnp.int32, (n, w), 1) + d0
        kvt = jnp.where(_head_of(row) == _head_of(col), gt_v[b, :n, :w], 0.0).astype(_bf16)
        mt = lax.dot_general(wo_v[lo:hi, :], kvt, _TN, preferred_element_type=_f32)
        mt_v[:, d0:d0 + w] = mt.astype(_bf16)
        zrow = gt_v[b, n:n + 1, :w]
        row = lax.broadcasted_iota(jnp.int32, (H, w), 0)
        col = lax.broadcasted_iota(jnp.int32, (H, w), 1) + d0
        zh_v[:, d0:d0 + w] = jnp.where(
            _head_of(col) == row, jnp.broadcast_to(zrow, (H, w)), 0.0).astype(_bf16)

    row = lax.broadcasted_iota(jnp.int32, (D, 2 * H), 0)
    col = lax.broadcasted_iota(jnp.int32, (D, 2 * H), 1)
    et_v[...] = jnp.where(_head_of(row) == (col & (H - 1)), 1.0, 0.0).astype(_bf16)

    def phase2a(i, carry):
        c0 = pl.multiple_of(i * TSA, TSA)
        pqt = pqt_v[:, pl.ds(c0, TSA)]
        den = jnp.dot(zh_v[...], pqt, preferred_element_type=_f32) + PHI_EPS
        rec = 1.0 / den
        hi = rec.astype(_bf16)
        lo = (rec - hi.astype(_f32)).astype(_bf16)
        hl = jnp.concatenate([hi, lo], axis=0)
        rexp = jnp.dot(et_v[...], hl, preferred_element_type=_f32)
        at = (pqt.astype(_f32) * rexp).astype(_bf16)
        attn = jnp.dot(mt_v[...], at, preferred_element_type=_f32)
        ht = xt_v[:, pl.ds(c0, TSA)].astype(_f32) + attn
        b2c = jnp.concatenate([b2c_v[...]] * (TSA // 128), axis=1)
        res_v[:, pl.ds(c0, TSA)] = ht + b2c
        lnt = _layernorm_t(ht)
        prow = lax.broadcasted_iota(jnp.int32, (DP - D, TSA), 0)
        lnt = jnp.concatenate([lnt, jnp.where(prow == 0, 1.0, 0.0)], axis=0)
        ln2_v[pl.ds(c0, TSA), :] = jnp.transpose(lnt).astype(_bf16)
        return carry

    lax.fori_loop(0, NBA, phase2a, 0)

    w1_copy.wait()
    w2_copy.wait()

    def ffn_block(i, carry):
        r0 = pl.multiple_of(i * TSF, TSF)
        hp = jnp.dot(ln2_v[pl.ds(r0, TSF), :], w1_v[...], preferred_element_type=_f32)
        r = jnp.maximum(hp, 0.0)
        hid = (r * r).astype(_bf16)
        y = lax.dot_general(w2t_v[...], hid, _NT, preferred_element_type=_f32)
        ot_v[:, pl.ds(r0, TSF)] = (res_v[:, pl.ds(r0, TSF)] + y).astype(_bf16)
        o_copy(i).start()
        return carry

    lax.fori_loop(0, NBF, ffn_block, 0)

    for i in range(NBF):
        o_copy(i).wait()


@jax.jit
def pallas_sequential_preLN__linear_attn_block__dense_activation_squared_relu__prompt_kernel(
    A_x: jax.Array,
    A_wqkv: jax.Array,
    A_wo: jax.Array,
    B_x: jax.Array,
    B_w1: jax.Array,
    B_b1: jax.Array,
    B_w2: jax.Array,
    B_b2: jax.Array,
):
    del B_x
    xt = jnp.transpose(A_x.reshape(S, D))
    w2t = jnp.transpose(B_w2)

    hbm_spec = pl.BlockSpec(memory_space=pltpu.HBM)
    vmem_spec = pl.BlockSpec(memory_space=pltpu.VMEM)

    outt = pl.pallas_call(
        _kernel,
        out_shape=jax.ShapeDtypeStruct((D, S), _bf16),
        in_specs=[hbm_spec, hbm_spec, hbm_spec, hbm_spec, vmem_spec, hbm_spec, vmem_spec],
        out_specs=hbm_spec,
        scratch_shapes=[
            pltpu.VMEM((D, S), _bf16),
            pltpu.VMEM((D, 3 * D), _bf16),
            pltpu.VMEM((3 * D, D), _bf16),
            pltpu.VMEM((D, D), _bf16),
            pltpu.VMEM((DP, F), _bf16),
            pltpu.VMEM((D, F), _bf16),
            pltpu.VMEM((D, S), _bf16),
            pltpu.VMEM((D, S), _bf16),
            pltpu.VMEM((len(_PIECES), _PROWS, 128), _f32),
            pltpu.VMEM((D, D), _bf16),
            pltpu.VMEM((H, D), _bf16),
            pltpu.VMEM((D, 2 * H), _bf16),
            pltpu.VMEM((D, 128), _f32),
            pltpu.VMEM((S, DP), _bf16),
            pltpu.VMEM((D, S), _f32),
            pltpu.SemaphoreType.DMA((NB1,)),
            pltpu.SemaphoreType.DMA((3,)),
            pltpu.SemaphoreType.DMA((NBF,)),
            pltpu.SemaphoreType.DMA((len(_WCH),)),
        ],
        compiler_params=pltpu.CompilerParams(vmem_limit_bytes=100 * 1024 * 1024),
    )(xt, A_wqkv, A_wo, B_w1, B_b1, w2t, B_b2)
    return jnp.transpose(outt).reshape(1, S, D)
```

```python
import jax
import jax.numpy as jnp
from jax import lax
import jax.experimental.pallas as pl
import jax.experimental.pallas.tpu as pltpu

S = 2048
D = 576
F = 4608
H = 32
DH = D // H
DP = 640
LN_EPS = 1e-5
PHI_EPS = 1e-6

TS1 = 512
TSA = 2048
TSF = 256

NB1 = S // TS1
NBA = S // TSA
NBF = S // TSF
ONES_ROWS = 16

_PIECES = []
for _b in range(0, D, 128):
    _w = min(128, D - _b)
    _lo = ((_b // DH) * DH) // 16 * 16
    _hi = -(-((((_b + _w - 1) // DH) + 1) * DH) // 16) * 16
    _PIECES.append((_b, _w, _lo, _hi))
_PROWS = max(hi - lo for _, _, lo, hi in _PIECES) + ONES_ROWS
_WCH = [(c, min(512, 3 * D - c)) for c in range(0, 3 * D, 512)]

_f32 = jnp.float32
_bf16 = jnp.bfloat16
_NT = (((1,), (1,)), ((), ()))
_TN = (((0,), (0,)), ((), ()))


def _layernorm_t(xt):
    m = jnp.mean(xt, axis=0, keepdims=True)
    xc = xt - m
    v = jnp.mean(xc * xc, axis=0, keepdims=True)
    return xc * lax.rsqrt(v + LN_EPS)


def _head_of(idx):
    return jnp.floor((idx.astype(_f32) + 0.5) * (1.0 / DH)).astype(jnp.int32)


def _kernel(xt_hbm, wqkv_hbm, wo_hbm, w1_hbm, b1_ref, w2t_hbm, b2_ref, ot_hbm,
            xt_v, wqkv_v, wqkvt_v, wo_v, w1_v, w2t_v, pqt_v, ot_v, gt_v, mt_v, zh_v, rec_v, b2c_v,
            ln2_v, res_v,
            sem_x, sem_w, sem_o, sem_q):
    def x_copy(i):
        return pltpu.make_async_copy(
            xt_hbm.at[:, pl.ds(i * TS1, TS1)], xt_v.at[:, pl.ds(i * TS1, TS1)], sem_x.at[i])

    def o_copy(i):
        return pltpu.make_async_copy(
            ot_v.at[:, pl.ds(i * TSF, TSF)], ot_hbm.at[:, pl.ds(i * TSF, TSF)], sem_o.at[i])

    def wqkv_copy(j):
        c, w = _WCH[j]
        return pltpu.make_async_copy(
            wqkv_hbm.at[:, pl.ds(c, w)], wqkv_v.at[:, pl.ds(c, w)], sem_q.at[j])

    wo_copy = pltpu.make_async_copy(wo_hbm, wo_v, sem_w.at[0])
    w1_copy = pltpu.make_async_copy(w1_hbm, w1_v.at[pl.ds(0, D), :], sem_w.at[1])
    w2_copy = pltpu.make_async_copy(w2t_hbm, w2t_v, sem_w.at[2])

    for j in range(len(_WCH)):
        wqkv_copy(j).start()
    x_copy(0).start()

    gt_v[...] = jnp.zeros(gt_v.shape, _f32)
    brow = lax.broadcasted_iota(jnp.int32, (DP - D, F), 0)
    w1_v[D:, :] = jnp.where(
        brow == 0, jnp.broadcast_to(b1_ref[...].astype(_f32).reshape(1, F), (DP - D, F)),
        0.0).astype(_bf16)
    b2pad = jnp.concatenate(
        [b2_ref[...].astype(_f32).reshape(1, D), jnp.zeros((1, DP - D), _f32)], axis=1)
    b2c_v[...] = jnp.transpose(jnp.broadcast_to(b2pad, (128, DP)))[:D, :]

    eye_r = lax.broadcasted_iota(jnp.int32, (128, 128), 0)
    eye_c = lax.broadcasted_iota(jnp.int32, (128, 128), 1)
    eye = jnp.where(eye_r == eye_c, 1.0, 0.0).astype(_bf16)
    for j, (c0, wc) in enumerate(_WCH):
        wqkv_copy(j).wait()
        if j == len(_WCH) - 1:
            for i in range(1, NB1):
                x_copy(i).start()
            wo_copy.start()
            w1_copy.start()
            w2_copy.start()
        for c in range(c0, c0 + wc, 128):
            w = min(128, 3 * D - c)
            t = lax.dot_general(eye[:w, :w], wqkv_v[:, c:c + w], _NT, preferred_element_type=_f32)
            wqkvt_v[c:c + w, :] = t.astype(_bf16)

    def phase1(i, carry):
        x_copy(i).wait()
        c0 = pl.multiple_of(i * TS1, TS1)
        xt = xt_v[:, pl.ds(c0, TS1)].astype(_f32)
        lnt = _layernorm_t(xt).astype(_bf16)
        qkvt = jnp.dot(wqkvt_v[...], lnt, preferred_element_type=_f32)
        qk = qkvt[:2 * D]
        p = (jnp.where(qk > 0, qk + 1.0, jnp.exp(qk)) + PHI_EPS).astype(_bf16)
        pqt_v[:, pl.ds(c0, TS1)] = p[:D]
        pkt = p[D:]
        vt = qkvt[2 * D:].astype(_bf16)
        ones = jnp.ones((ONES_ROWS, TS1), _bf16)
        for b, (d0, w, lo, hi) in enumerate(_PIECES):
            lhs = jnp.concatenate([vt[lo:hi], ones], axis=0)
            gt_v[b, :hi - lo + ONES_ROWS, :w] += lax.dot_general(
                lhs, pkt[d0:d0 + w], _NT, preferred_element_type=_f32)
        return carry

    lax.fori_loop(0, NB1, phase1, 0)

    wo_copy.wait()
    for b, (d0, w, lo, hi) in enumerate(_PIECES):
        n = hi - lo
        row = lax.broadcasted_iota(jnp.int32, (n, w), 0) + lo
        col = lax.broadcasted_iota(jnp.int32, (n, w), 1) + d0
        kvt = jnp.where(_head_of(row) == _head_of(col), gt_v[b, :n, :w], 0.0).astype(_bf16)
        mt = lax.dot_general(wo_v[lo:hi, :], kvt, _TN, preferred_element_type=_f32)
        mt_v[:, d0:d0 + w] = mt.astype(_bf16)
        zrow = gt_v[b, n:n + 1, :w]
        row = lax.broadcasted_iota(jnp.int32, (H, w), 0)
        col = lax.broadcasted_iota(jnp.int32, (H, w), 1) + d0
        zh_v[:, d0:d0 + w] = jnp.where(
            _head_of(col) == row, jnp.broadcast_to(zrow, (H, w)), 0.0).astype(_bf16)

    def phase2a(i, carry):
        c0 = pl.multiple_of(i * TSA, TSA)
        pqt = pqt_v[:, pl.ds(c0, TSA)]
        den = jnp.dot(zh_v[...], pqt, preferred_element_type=_f32) + PHI_EPS
        rec_v[...] = 1.0 / den
        sub = lax.broadcasted_iota(jnp.int32, (8, TSA), 0)
        groups = []
        for g in range(D // 8):
            h1, h2 = (8 * g) // DH, (8 * g + 7) // DH
            r1 = jnp.broadcast_to(rec_v[h1:h1 + 1, :], (8, TSA))
            if h2 != h1:
                r2 = jnp.broadcast_to(rec_v[h2:h2 + 1, :], (8, TSA))
                r1 = jnp.where(sub < h2 * DH - 8 * g, r1, r2)
            groups.append(r1)
        rexp = jnp.concatenate(groups, axis=0)
        at = (pqt.astype(_f32) * rexp).astype(_bf16)
        attn = jnp.dot(mt_v[...], at, preferred_element_type=_f32)
        ht = xt_v[:, pl.ds(c0, TSA)].astype(_f32) + attn
        b2c = jnp.concatenate([b2c_v[...]] * (TSA // 128), axis=1)
        res_v[:, pl.ds(c0, TSA)] = ht + b2c
        lnt = _layernorm_t(ht)
        prow = lax.broadcasted_iota(jnp.int32, (DP - D, TSA), 0)
        lnt = jnp.concatenate([lnt, jnp.where(prow == 0, 1.0, 0.0)], axis=0)
        ln2_v[pl.ds(c0, TSA), :] = jnp.transpose(lnt).astype(_bf16)
        return carry

    lax.fori_loop(0, NBA, phase2a, 0)

    w1_copy.wait()
    w2_copy.wait()

    def ffn_block(i, carry):
        r0 = pl.multiple_of(i * TSF, TSF)
        hp = jnp.dot(ln2_v[pl.ds(r0, TSF), :], w1_v[...], preferred_element_type=_f32)
        r = jnp.maximum(hp, 0.0)
        hid = (r * r).astype(_bf16)
        y = lax.dot_general(w2t_v[...], hid, _NT, preferred_element_type=_f32)
        ot_v[:, pl.ds(r0, TSF)] = (res_v[:, pl.ds(r0, TSF)] + y).astype(_bf16)
        o_copy(i).start()
        return carry

    lax.fori_loop(0, NBF, ffn_block, 0)

    for i in range(NBF):
        o_copy(i).wait()


@jax.jit
def pallas_sequential_preLN__linear_attn_block__dense_activation_squared_relu__prompt_kernel(
    A_x: jax.Array,
    A_wqkv: jax.Array,
    A_wo: jax.Array,
    B_x: jax.Array,
    B_w1: jax.Array,
    B_b1: jax.Array,
    B_w2: jax.Array,
    B_b2: jax.Array,
):
    del B_x
    xt = jnp.transpose(A_x.reshape(S, D))
    w2t = jnp.transpose(B_w2)

    hbm_spec = pl.BlockSpec(memory_space=pltpu.HBM)
    vmem_spec = pl.BlockSpec(memory_space=pltpu.VMEM)

    outt = pl.pallas_call(
        _kernel,
        out_shape=jax.ShapeDtypeStruct((D, S), _bf16),
        in_specs=[hbm_spec, hbm_spec, hbm_spec, hbm_spec, vmem_spec, hbm_spec, vmem_spec],
        out_specs=hbm_spec,
        scratch_shapes=[
            pltpu.VMEM((D, S), _bf16),
            pltpu.VMEM((D, 3 * D), _bf16),
            pltpu.VMEM((3 * D, D), _bf16),
            pltpu.VMEM((D, D), _bf16),
            pltpu.VMEM((DP, F), _bf16),
            pltpu.VMEM((D, F), _bf16),
            pltpu.VMEM((D, S), _bf16),
            pltpu.VMEM((D, S), _bf16),
            pltpu.VMEM((len(_PIECES), _PROWS, 128), _f32),
            pltpu.VMEM((D, D), _bf16),
            pltpu.VMEM((H, D), _bf16),
            pltpu.VMEM((H, TSA), _f32),
            pltpu.VMEM((D, 128), _f32),
            pltpu.VMEM((S, DP), _bf16),
            pltpu.VMEM((D, S), _f32),
            pltpu.SemaphoreType.DMA((NB1,)),
            pltpu.SemaphoreType.DMA((3,)),
            pltpu.SemaphoreType.DMA((NBF,)),
            pltpu.SemaphoreType.DMA((len(_WCH),)),
        ],
        compiler_params=pltpu.CompilerParams(vmem_limit_bytes=100 * 1024 * 1024),
    )(xt, A_wqkv, A_wo, B_w1, B_b1, w2t, B_b2)
    return jnp.transpose(outt).reshape(1, S, D)
```
